```python
import os as _os
_os.environ.setdefault("JAX_PLATFORMS", "cpu")
import jax
import jax.numpy as jnp

def _softmax(x, axis=-1):
    return jax.nn.softmax(x, axis=axis)
def _gelu(x):
    return jax.nn.gelu(x, approximate=True)
def _silu(x):
    return jax.nn.silu(x)
def _sigmoid(x):
    return jax.nn.sigmoid(x)
def _layernorm(x, axis=-1, eps=1e-5):
    m = jnp.mean(x, axis=axis, keepdims=True)
    v = jnp.var(x, axis=axis, keepdims=True)
    return (x - m) / jnp.sqrt(v + eps)
def _scatter_add(tgt, idx, src, axis=0):
    return tgt.at[idx].add(src)
def _segment_sum(src, seg, n):
    return jax.ops.segment_sum(src, seg, n)
class _Rng:
    def __init__(self, key):
        self._k = key
    def _next(self):
        self._k, sub = jax.random.split(self._k)
        return sub
    def normal(self, shape):
        return jax.random.normal(self._next(), shape, dtype=jnp.bfloat16)
    def randint(self, lo, hi, shape):
        return jax.random.randint(self._next(), shape, lo, hi, dtype=jnp.int32)
    def uniform(self, shape, lo=0.0, hi=1.0):
        return jax.random.uniform(self._next(), shape, jnp.bfloat16, lo, hi)
    def permutation(self, n):
        return jax.random.permutation(self._next(), n)


kernel_name = 'gated_mix__softmax_full_mha__dense_activation_relu__prompt'

def setup_inputs():
    _rng = _Rng(jax.random.key(int.from_bytes(__import__("os").urandom(4), "little")))
    _w = (lambda a: (lambda t: t.astype(jnp.bfloat16) if jnp.issubdtype(t.dtype, jnp.floating) else t)(jnp.asarray(a)))
    def _A_setup():
        B, S, D = 1, 2048, 640
        return {
            "x": _w((lambda *s: _rng.normal(s) * 0.05)(B, S, D)),
            "wqkv": _w((lambda *s: _rng.normal(s) * 0.8)(D, 3 * D)),
            "wo": _w((lambda *s: _rng.normal(s) * 0.05)(D, D)),
        }
    _A_in = _A_setup()

    def _B_setup():
        B, S, D, Dff = 1, 2048, 640, 1536
        return {
            "x": _w((lambda *s: _rng.normal(s) * 0.05)(B, S, D)),
            "w1": _w((lambda *s: _rng.normal(s) * 0.05)(D, Dff)),
            "w2": _w((lambda *s: _rng.normal(s) * 0.05)(Dff, D)),
        }
    _B_in = _B_setup()

    return {
        "A_x": _A_in["x"],
        "A_wqkv": _A_in["wqkv"],
        "A_wo": _A_in["wo"],
        "B_x": _B_in["x"],
        "B_w1": _B_in["w1"],
        "B_w2": _B_in["w2"],
        "gate_w": _w((lambda *s: _rng.normal(s) * 0.05)(640) * 16.0),
    }

def reference(A_x, A_wqkv, A_wo, B_x, B_w1, B_w2, gate_w):
    def _A_ref(x, wqkv, wo):
        B, S, D = x.shape
        H = 32; Dh = D // H
        qkv = (lambda x, *d: x.transpose(*d))((x @ wqkv).reshape(B, S, 3, H, Dh), 2, 0, 3, 1, 4)
        q, k, v = qkv[0], qkv[1], qkv[2]
        scale = Dh ** -0.5
        scores = jnp.einsum("bhqd,bhkd->bhqk", q, k) * scale
        p = _softmax(scores, axis=-1)
        o = jnp.einsum("bhqk,bhkd->bhqd", p, v)
        return (lambda x, *d: x.transpose(*d))(o, 0, 2, 1, 3).reshape(B, S, D) @ wo

    def _B_ref(x, w1, w2):
        h = jnp.einsum("bsd,df->bsf", x, w1)
        zero = jnp.zeros_like(h)
        h = jnp.maximum(h, zero)
        return jnp.einsum("bsf,fd->bsd", h, w2)

    x = A_x
    g = _sigmoid((x * gate_w).sum(-1, keepdims=True))
    a = _A_ref(x, A_wqkv, A_wo)
    b = _B_ref(x, B_w1, B_w2)
    return g * a + (1 - g) * b
```

```python
import functools
import numpy as np
import jax
import jax.numpy as jnp
from jax import lax
import jax.experimental.pallas as pl
import jax.experimental.pallas.tpu as pltpu

_NN = (((1,), (0,)), ((), ()))
_NT = (((1,), (1,)), ((), ()))
_H = 32
_LANES = 128


def _dot(a, b, dims=_NN):
    return lax.dot_general(a, b, dims, preferred_element_type=jnp.float32)


def _kernel(x_ref, wqkv_ref, wo_ref, w1_ref, w2_ref, gw_ref, o_ref,
            wt_scr, k_scr, qt_scr, vt_scr, s_scr, ot_scr, *, bq, kc, bm, unroll):
    f32, bf16 = jnp.float32, jnp.bfloat16
    S, D = x_ref.shape
    dh = D // _H
    nt = D // _LANES
    qscale = np.float32(dh ** -0.5 * np.log2(np.e))

    wt_scr[0:D, :] = wqkv_ref[:, 0:D].T
    wt_scr[D:2 * D, :] = wqkv_ref[:, 2 * D:3 * D].T
    straddle = [h for h in range(_H) if (h * dh) // _LANES != (h * dh + dh - 1) // _LANES]

    def proj(i, c):
        r0 = pl.multiple_of(i * bm, bm)
        xb = x_ref[pl.ds(r0, bm), :]
        k = _dot(xb, wqkv_ref[:, D:2 * D])
        lane = lax.broadcasted_iota(jnp.int32, (bm, _LANES), 1)
        for j in range(nt):
            kj = k[:, j * _LANES:(j + 1) * _LANES]
            k_scr[2 * j, pl.ds(r0, bm), :] = kj.astype(bf16)
            if j + 1 < nt:
                kn = k[:, (j + 1) * _LANES:(j + 2) * _LANES]
                k_scr[2 * j + 1, pl.ds(r0, bm), :] = jnp.where(lane >= _LANES // 2, kj, kn).astype(bf16)
        qv = _dot(wt_scr[...], xb, _NT)
        qt_scr[0:D, pl.ds(r0, bm)] = (qv[0:D] * qscale).astype(bf16)
        v = qv[D:2 * D].astype(bf16).astype(f32)
        row = lax.broadcasted_iota(jnp.int32, (8, bm), 0)
        for t in range(_H // 2):
            b = t * 2 * dh
            mid = v[b + 16:b + 24]
            vt_scr[2 * t, :, pl.ds(r0, bm)] = jnp.concatenate(
                [v[b:b + 16], jnp.where(row < 4, mid, 1.0)], axis=0)
            vt_scr[2 * t + 1, :, pl.ds(r0, bm)] = jnp.concatenate(
                [jnp.where(row < 4, 1.0, mid), v[b + 24:b + 40]], axis=0)
        return c

    lax.fori_loop(0, S // bm, proj, 0)
    qt_scr[D:D + _LANES, :] = jnp.zeros((_LANES, S), bf16)

    nq = S // bq
    npair = _H // 2
    n_items = nq * _H
    urow = lax.broadcasted_iota(jnp.int32, (_LANES // 2, bq), 0)

    def masked_q(i):
        h = i % _H
        q0 = pl.multiple_of((i // _H) * bq, bq)
        c0 = h * dh
        j = c0 // _LANES
        lo = (c0 - j * _LANES) // 2
        hi = lo + dh // 2
        r = pl.multiple_of(j * _LANES, _LANES)
        a = pltpu.bitcast(qt_scr[pl.ds(r, _LANES), pl.ds(q0, bq)], jnp.uint32)
        b = pltpu.bitcast(qt_scr[pl.ds(r + _LANES, _LANES), pl.ds(q0, bq)], jnp.uint32)
        w = jnp.where((urow >= lo) & (urow < hi), a,
                      jnp.where(urow < hi - _LANES // 2, b, jnp.uint32(0)))
        kt = 2 * j + (hi > _LANES // 2).astype(jnp.int32)
        return pltpu.bitcast(w, bf16), kt

    def pass1(qm, kt, slot, j, m):
        s = _dot(k_scr[kt, j * kc:(j + 1) * kc, :], qm)
        s_scr[slot, j * kc:(j + 1) * kc, :] = s
        mj = jnp.max(s.reshape(kc // 8, 8, bq), axis=0)
        return mj if m is None else jnp.maximum(m, mj)

    def pass2(h, slot, j, m, acc):
        p = jnp.exp2(s_scr[slot, j * kc:(j + 1) * kc, :] - m).astype(bf16)
        pv = _dot(vt_scr[h, :, j * kc:(j + 1) * kc], p)
        return pv if acc is None else acc + pv

    qm, kt = masked_q(jnp.int32(0))
    m = None
    for j in range(S // kc):
        m = pass1(qm, kt, 0, j, m)
    m0 = jnp.max(m, axis=0, keepdims=True)
    row8 = lax.broadcasted_iota(jnp.int32, (8, bq), 0)

    def attn(tt, mprev):
        for w in range(unroll):
            t = tt * unroll + w
            outs = []
            for u in range(2):
                i = 2 * t + u
                qm, kt = masked_q(jnp.minimum(i + 1, n_items - 1))
                m = None
                acc = None
                for j in range(S // kc):
                    m = pass1(qm, kt, 1 - u, j, m)
                    acc = pass2(i % _H, u, j, mprev, acc)
                mprev = jnp.max(m, axis=0, keepdims=True)
                l = acc[20:21] if u == 0 else acc[0:1]
                outs.append(acc * (1.0 / l))
            e, o = outs
            q0 = pl.multiple_of((t // npair) * bq, bq)
            r0 = pl.multiple_of((t % npair) * 2 * dh, 8)
            ot_scr[pl.ds(r0, 2 * dh), pl.ds(q0, bq)] = jnp.concatenate(
                [e[0:16], jnp.where(row8 < 4, e[16:24], o[0:8]), o[8:24]], axis=0)
        return mprev

    lax.fori_loop(0, n_items // 2 // unroll, attn, m0)

    def tail(i, c):
        r0 = pl.multiple_of(i * bm, bm)
        xb = x_ref[pl.ds(r0, bm), :]
        hid = jnp.maximum(_dot(xb, w1_ref[...]), 0.0).astype(bf16)
        b = _dot(hid, w2_ref[...])
        o = ot_scr[:, pl.ds(r0, bm)].T.astype(bf16)
        a = _dot(o, wo_ref[...])
        z = jnp.sum(xb.astype(f32) * gw_ref[...].astype(f32), axis=-1, keepdims=True)
        g = jax.nn.sigmoid(z)
        o_ref[pl.ds(r0, bm), :] = (g * a + (1.0 - g) * b).astype(o_ref.dtype)
        return c

    lax.fori_loop(0, S // bm, tail, 0)


@jax.jit
def pallas_gated_mix__softmax_full_mha__dense_activation_relu__prompt_kernel(
    A_x, A_wqkv, A_wo, B_x, B_w1, B_w2, gate_w
):
    del B_x
    bq, kc, bm, unroll = 512, 128, 512, 2
    B, S, D = A_x.shape
    bf16, f32 = jnp.bfloat16, jnp.float32
    out = pl.pallas_call(
        functools.partial(_kernel, bq=bq, kc=kc, bm=bm, unroll=unroll),
        out_shape=jax.ShapeDtypeStruct((S, D), A_x.dtype),
        scratch_shapes=[
            pltpu.VMEM((2 * D, D), bf16),
            pltpu.VMEM((2 * (D // _LANES) - 1, S, _LANES), bf16),
            pltpu.VMEM((D + _LANES, S), bf16),
            pltpu.VMEM((_H, 24, S), f32),
            pltpu.VMEM((2, S, bq), f32),
            pltpu.VMEM((D, S), f32),
        ],
        compiler_params=pltpu.CompilerParams(vmem_limit_bytes=100 * 2**20),
    )(A_x.reshape(S, D), A_wqkv, A_wo, B_w1, B_w2, gate_w.reshape(1, D))
    return out.reshape(B, S, D)
```

```python
import numpy as np
import jax
import jax.numpy as jnp
from jax import lax
import jax.experimental.pallas as pl
import jax.experimental.pallas.tpu as pltpu

_H = 32
_L = 128
_VROWS = 24
_BQ = 512
_KC = 128
_BM = 512
_BQV = 1024
_ITEMS = 8
_LAG = 2
_EARLY = 48
_VPU = 128

_NN = (((1,), (0,)), ((), ()))
_NT = (((1,), (1,)), ((), ()))


def _dot(a, b, dims=_NN):
    return lax.dot_general(a, b, dims, preferred_element_type=jnp.float32)


def _tile(c):
    return slice(c * _L, (c + 1) * _L)


def _kernel(x_hbm, wqkv_hbm, wo_hbm, w1_hbm, w2_hbm, gw_hbm, o_hbm,
            x_v, wqkv_v, wo_v, w1_v, w2_v, gw_v,
            wt_s, k_s, qt_s, qm_s, vt_s, s_s, kb_s, ke_s, se_s, qo_s, qb_s, ev_s,
            one_s, b_s, x_sem, w_sem, o_sem):
    f32, bf16, u32 = jnp.float32, jnp.bfloat16, jnp.uint32
    S, D = x_v.shape
    F = w1_v.shape[1]
    dh = D // _H
    nt = D // _L
    nb = S // _BM
    hl = _L // 2

    def paced(keep, value, after):
        return jnp.where(keep, value, after)

    def x_copy(i):
        rows = pl.ds(pl.multiple_of(i * _BM, _BM), _BM)
        return pltpu.make_async_copy(x_hbm.at[rows], x_v.at[rows], x_sem.at[i])

    wq_cp, wk_cp, wv_cp = [
        pltpu.make_async_copy(wqkv_hbm.at[:, pl.ds(j * D, D)], wqkv_v.at[j], w_sem.at[j])
        for j in range(3)]
    late_cp = [
        pltpu.make_async_copy(src, dst, w_sem.at[3 + j]) for j, (src, dst) in enumerate(
            ((w1_hbm, w1_v), (w2_hbm, w2_v), (wo_hbm, wo_v), (gw_hbm, gw_v)))]
    wk_cp.start()
    x_copy(0).start()
    qt_s[D // 2:D // 2 + hl, :] = jnp.zeros((hl, S), u32)
    s_s[1] = jnp.zeros((S, _BQ), f32)
    ev_s[...] = jnp.ones(ev_s.shape, f32)
    one_s[...] = jnp.ones(one_s.shape, jnp.int32)
    wk_cp.wait()

    def k_proj(i, carry):
        x_copy(i).wait()

        @pl.when(i < nb - 1)
        def _():
            x_copy(i + 1).start()

        pl.when(i == 0)(wq_cp.start)
        pl.when(i == 1)(wv_cp.start)
        pl.when(i == nb - 2)(wq_cp.wait)

        @pl.when(i == nb - 1)
        def _():
            wv_cp.wait()
            for cp in late_cp:
                cp.start()

        src = jnp.where(i == nb - 2, 0, jnp.where(i == nb - 1, 2, 1))
        wt_s[jnp.where(i == nb - 1, 1, 0)] = wqkv_v[src].T
        upper = lax.broadcasted_iota(jnp.int32, (_L, _L), 1) >= hl
        for a in range(_BM // _L):
            r0 = pl.multiple_of(i * _BM + a * _L, _L)
            pairs = pl.ds(pl.multiple_of(r0 // 2, hl), hl)
            k = _dot(x_v[pl.ds(r0, _L), :], wqkv_v[1])
            for j in range(nt):
                k_s[2 * j, pairs, :] = pltpu.bitcast(k[:, _tile(j)].astype(bf16), u32)
                if j + 1 < nt:
                    mixed = jnp.where(upper, k[:, _tile(j)], k[:, _tile(j + 1)])
                    k_s[2 * j + 1, pairs, :] = pltpu.bitcast(mixed.astype(bf16), u32)
        return carry

    lax.fori_loop(0, nb, k_proj, 0)

    def spread_keys(dst, rows, j, packed):
        for l in range(_L):
            col = jnp.broadcast_to(packed[:, l:l + 1], packed.shape)
            dst[j * _L + l, rows, :] = pltpu.bitcast(col, bf16).astype(f32)

    def qv_proj(i, carry):
        tok = pl.ds(pl.multiple_of(i * _BQV, _BQV), _BQV)
        xb = x_v[tok, :]
        n = 16 * pl.cdiv(_EARLY // 16, S // _BQV)
        e0 = pl.multiple_of(jnp.minimum(i * n, _EARLY - n), 16)
        for j in range(nt):
            spread_keys(ke_s, pl.ds(e0, n), j,
                        k_s[2 * j, pl.ds(pl.multiple_of(e0 // 2, 8), n // 2), :])
        v = _dot(wt_s[1], xb, _NT).astype(bf16).astype(f32)
        low = lax.broadcasted_iota(jnp.int32, (8, _BQV), 0) < 4
        for t in range(_H // 2):
            r = t * 2 * dh
            mid = v[r + 16:r + 24]
            vt_s[2 * t, :, tok] = jnp.concatenate(
                [v[r:r + 16], jnp.where(low, mid, 1.0)], axis=0)
            vt_s[2 * t + 1, :, tok] = jnp.concatenate(
                [jnp.where(low, 1.0, mid), v[r + 24:r + 40]], axis=0)
        scale = np.float32(dh ** -0.5 * np.log2(np.e))
        q = (_dot(wt_s[0], xb, _NT) * scale).astype(bf16)
        qt_s[0:D // 2, tok] = pltpu.bitcast(q, u32)
        qo_s[:, tok] = q.astype(f32)
        return carry

    lax.fori_loop(0, S // _BQV, qv_proj, 0)
    for cp in late_cp:
        cp.wait()

    fw = 4 * _L
    heads = _H // nb
    e_steps = [(h, c, d) for h in range(heads) for c in range(S // _L) for d in range(dh)]
    n_dots = 2 * (F // fw) * nt
    e_cut = [len(e_steps) * min(j, n_dots - 1) // (n_dots - 1) for j in range(n_dots + 1)]

    def ffn(i, carry):
        rows = pl.ds(pl.multiple_of(i * _BM, _BM), _BM)
        keep = one_s[...] != 0
        state = {"dot": 0}

        def dot_and_scores(a, b):
            res = _dot(a, b)
            steps = e_steps[e_cut[state["dot"]]:e_cut[state["dot"] + 1]]
            state["dot"] += 1
            for n, (h, c, d) in enumerate(steps):
                r = h * dh + d
                if d == 0 or r % 8 == 0 or n % 4 == 0:
                    r8 = pl.multiple_of(i * heads * dh + r // 8 * 8, 8)
                    o = 8 * (_BM // 8 * n // len(steps))
                    state["q"] = paced(keep, qo_s[pl.ds(r8, 8), _tile(c)], res[o:o + 8, 0:_L])
                term = ke_s[i * heads * dh + r] * state["q"][r % 8:r % 8 + 1]
                state["s"] = term if d == 0 else state["s"] + term
                if d == dh - 1:
                    se_s[i * heads + h, :, _tile(c)] = state["s"]
            return res

        hid = []
        for n in range(F // fw):
            rest = dot_and_scores(x_v[rows, fw:D], w1_v[fw:D, n * fw:(n + 1) * fw])
            cols = []
            for c in range(fw // _L):
                head = dot_and_scores(x_v[rows, 0:fw], w1_v[0:fw, _tile(n * fw // _L + c)])
                cols.append(jnp.maximum(head + rest[:, _tile(c)], 0.0).astype(bf16))
            hid.append(jnp.concatenate(cols, axis=1))
        nk = _VPU // nb
        v0 = pl.multiple_of(i * nk, nk)
        for j in range(nt):
            acc = None
            for n in range(F // fw):
                part = dot_and_scores(hid[n], w2_v[n * fw:(n + 1) * fw, _tile(j)])
                acc = part if n == 0 else acc + part
                if n == 0:
                    packed = k_s[2 * j, pl.ds(pl.multiple_of((_EARLY + v0) // 2, 8), nk // 2), :]
                    spread_keys(kb_s, pl.ds(v0, nk), j, paced(
                        jnp.concatenate([one_s[...]] * (nk // 16), axis=0) != 0, packed,
                        pltpu.bitcast(part[_BM - nk // 2:_BM], u32)))
            b_s[rows, _tile(j)] = acc
        return carry

    lax.fori_loop(0, nb, ffn, 0)

    nch = S // _KC
    nqt = _BQ // _L
    n_items = (S // _BQ) * _H
    first = _EARLY + _VPU
    k_cut = [first + 16 * ((S - first) // 16 * j // nch) for j in range(nch + 1)]
    v_steps = [(r, d) for r in range(0, _VPU, 8) for d in range(dh)]
    v_cut = [len(v_steps) * j // nch for j in range(nch + 1)]
    v_cut0 = [len(v_steps) * max(j - 2, 0) // (nch - 2) for j in range(nch + 1)]

    def queries(i):
        return pl.ds(pl.multiple_of((i // _H) * _BQ, _BQ), _BQ)

    def head_span(i):
        c0 = (i % _H) * dh
        j = c0 // _L
        lo = (c0 - j * _L) // 2
        return j, lo, lo + dh // 2

    def k_tile(i):
        j, _, hi = head_span(i)
        return 2 * j + (hi > hl).astype(jnp.int32)

    def mask_q(i, slot):
        j, lo, hi = head_span(i)
        r = pl.multiple_of(j * hl, hl)
        pair = lax.broadcasted_iota(jnp.int32, (hl, _BQ), 0)
        qm_s[slot] = jnp.where(
            (pair >= lo) & (pair < hi), qt_s[pl.ds(r, hl), queries(i)],
            jnp.where(pair < hi - hl, qt_s[pl.ds(r + hl, hl), queries(i)], u32(0)))

    def paced_rows(keep, value, after):
        return jnp.concatenate(
            [paced(keep, value[:, _tile(c)], after[8 * c:8 * c + 8, 0:_L]) for c in range(nqt)],
            axis=1)

    def spread_q(i, slot, dims, keep=None, after=None):
        base = ((i % _H) // 2) * 2 * dh
        for d in dims:
            r = slot * dh + d
            q8 = qo_s[pl.ds(pl.multiple_of(base + r // 8 * 8, 8), 8), queries(i)]
            if after is not None:
                q8 = paced_rows(keep, q8, after)
            qb_s[slot, d] = jnp.broadcast_to(q8[r % 8:r % 8 + 1], (8, _BQ))

    def put_scores(slot, r0, s, m):
        s_s[slot, r0:r0 + s.shape[0], :] = s
        top = jnp.max(s.reshape(s.shape[0] // 8, 8, _BQ), axis=0)
        return top if m is None else jnp.maximum(m, top)

    def probs_times_v(h, slot, j, m):
        keys = slice(j * _KC, (j + 1) * _KC)
        p = jnp.exp2(s_s[slot, keys, :] - m).astype(bf16)
        return _dot(vt_s[h, :, keys], p)

    def finish(i, odd_head, acc):
        if not odd_head:
            ev_s[...] = acc
            return
        even = ev_s[...] * (1.0 / ev_s[dh:dh + 1])
        odd = acc * (1.0 / acc[0:1])
        low = lax.broadcasted_iota(jnp.int32, (8, _BQ), 0) < 4
        r0 = pl.multiple_of(((i % _H) // 2) * 2 * dh, 8)
        qo_s[pl.ds(r0, 2 * dh), queries(i)] = jnp.concatenate(
            [even[0:16], jnp.where(low, even[16:24], odd[0:8]), odd[8:24]], axis=0)

    def attend(t, carry):
        m_in, kt = carry
        keep = one_s[...] != 0
        maxes = [m_in]
        m = prev = part = acc = m_row = None
        for c in range(_ITEMS * nch + _LAG):
            if c < _ITEMS * nch:
                n, j = divmod(c, nch)
                i, slot = t * _ITEMS + n, n % 2
                nxt = jnp.minimum(i + 1, n_items - 1)
                if j == 0:
                    m = None
                cut = v_cut if n else v_cut0
                steps = v_steps[cut[j]:cut[j + 1]]
                for a, (r, d) in enumerate(steps):
                    kd = kb_s[(i % _H) * dh + d, r:r + 8, :]
                    if a % 3 == 0:
                        o = 8 * int(prev.shape[0] // 8 * (6 + 10 * a / len(steps)) / 16)
                        kd = paced(keep, kd, prev[o:o + 8, 0:_L])
                    term = jnp.concatenate([kd] * nqt, axis=1) * qb_s[slot, d]
                    part = term if d == 0 else part + term
                    if d == dh - 1:
                        m = put_scores(slot, _EARLY + r, part, m)
                if 4 <= j < 4 + dh // 2:
                    spread_q(nxt, 1 - slot, (2 * (j - 4), 2 * (j - 4) + 1), keep, prev)
                if 6 <= j < 6 + _EARLY // 8:
                    r = (j - 6) * 8
                    early = paced_rows(keep, se_s[i % _H, r:r + 8, queries(i)], prev)
                    m = put_scores(slot, r, early, m)
                if j == nch - 2:
                    mask_q(nxt, 1 - slot)
                k = pltpu.bitcast(k_s[kt, k_cut[j] // 2:k_cut[j + 1] // 2, :], bf16)
                prev = _dot(k, pltpu.bitcast(qm_s[slot], bf16))
                m = put_scores(slot, k_cut[j], prev, m)
                if j == nch - 1:
                    maxes.append(m)
                    kt = k_tile(nxt)
            if c >= _LAG:
                n, j = divmod(c - _LAG, nch)
                i = jnp.abs(t * _ITEMS + n - 1)
                if j == 0:
                    m_row = jnp.max(maxes[n], axis=0, keepdims=True)
                pv = probs_times_v(i % _H, 1 - n % 2, j, m_row)
                acc = pv if j == 0 else acc + pv
                if j == nch - 1:
                    finish(i, n % 2 == 0, acc)
        return maxes[_ITEMS], kt

    mask_q(jnp.int32(0), 0)
    spread_q(jnp.int32(0), 0, range(dh))
    m_last, _ = lax.fori_loop(
        0, n_items // _ITEMS, attend, (jnp.zeros((8, _BQ), f32), jnp.int32(0)))
    m_row = jnp.max(m_last, axis=0, keepdims=True)
    acc = None
    for j in range(nch):
        pv = probs_times_v(_H - 1, 1, j, m_row)
        acc = pv if j == 0 else acc + pv
    finish(jnp.int32(n_items - 1), True, acc)

    out_cp = []
    for a in range(S // _L):
        rows = pl.ds(a * _L, _L)
        att = _dot(qo_s[:, rows].T.astype(bf16), wo_v[...])
        z = jnp.sum(x_v[rows, :].astype(f32) * gw_v[...].astype(f32), axis=-1, keepdims=True)
        gate = jax.nn.sigmoid(z)
        x_v[rows, :] = (gate * att + (1.0 - gate) * b_s[rows, :]).astype(x_v.dtype)
        out_cp.append(pltpu.make_async_copy(x_v.at[rows], o_hbm.at[rows], o_sem.at[a]))
        out_cp[-1].start()
    for cp in out_cp:
        cp.wait()


@jax.jit
def pallas_gated_mix__softmax_full_mha__dense_activation_relu__prompt_kernel(
    A_x: jax.Array,
    A_wqkv: jax.Array,
    A_wo: jax.Array,
    B_x: jax.Array,
    B_w1: jax.Array,
    B_w2: jax.Array,
    gate_w: jax.Array,
):
    del B_x
    B, S, D = A_x.shape
    F = B_w1.shape[1]
    assert (B, S, D, F) == (1, 2048, 640, 1536)
    bf16, f32, u32 = jnp.bfloat16, jnp.float32, jnp.uint32
    hbm = pl.BlockSpec(memory_space=pl.ANY)
    out = pl.pallas_call(
        _kernel,
        out_shape=jax.ShapeDtypeStruct((S, D), bf16),
        in_specs=[hbm] * 6,
        out_specs=hbm,
        scratch_shapes=[
            pltpu.VMEM((S, D), bf16),
            pltpu.VMEM((3, D, D), bf16),
            pltpu.VMEM((D, D), bf16),
            pltpu.VMEM((D, F), bf16),
            pltpu.VMEM((F, D), bf16),
            pltpu.VMEM((D,), bf16),
            pltpu.VMEM((2, D, D), bf16),
            pltpu.VMEM((2 * (D // _L) - 1, S // 2, _L), u32),
            pltpu.VMEM(((D + _L) // 2, S), u32),
            pltpu.VMEM((2, _L // 2, _BQ), u32),
            pltpu.VMEM((_H, _VROWS, S), f32),
            pltpu.VMEM((2, S, _BQ), f32),
            pltpu.VMEM((D, _VPU, _L), f32),
            pltpu.VMEM((D, _EARLY, _L), f32),
            pltpu.VMEM((_H, _EARLY, S), f32),
            pltpu.VMEM((D, S), f32),
            pltpu.VMEM((2, D // _H, 8, _BQ), f32),
            pltpu.VMEM((_VROWS, _BQ), f32),
            pltpu.VMEM((8, _L), jnp.int32),
            pltpu.VMEM((S, D), f32),
            pltpu.SemaphoreType.DMA((S // _BM,)),
            pltpu.SemaphoreType.DMA((7,)),
            pltpu.SemaphoreType.DMA((S // _L,)),
        ],
        compiler_params=pltpu.CompilerParams(vmem_limit_bytes=124 * 2**20),
    )(A_x.reshape(S, D), A_wqkv, A_wo, B_w1, B_w2, gate_w)
    return out.reshape(B, S, D)
```

```python
import numpy as np
import jax
import jax.numpy as jnp
from jax import lax
import jax.experimental.pallas as pl
import jax.experimental.pallas.tpu as pltpu

_H = 32
_L = 128
_VROWS = 24
_BQ = 512
_KC = 128
_BM = 512
_BQV = 1024
_ITEMS = 8
_LAG = 2
_EARLY = 48
_VPU = 128

_NN = (((1,), (0,)), ((), ()))
_NT = (((1,), (1,)), ((), ()))


def _dot(a, b, dims=_NN):
    return lax.dot_general(a, b, dims, preferred_element_type=jnp.float32)


def _tile(c):
    return slice(c * _L, (c + 1) * _L)


def _kernel(x_hbm, wqkv_hbm, wo_hbm, w1_hbm, w2_hbm, gw_hbm, o_hbm,
            x_v, wqkv_v, wo_v, w1_v, w2_v, gw_v,
            wt_s, k_s, qt_s, qm_s, vt_s, s_s, kb_s, ke_s, se_s, qo_s, qb_s, ev_s,
            one_s, b_s, x_sem, w_sem, o_sem):
    f32, bf16, u32 = jnp.float32, jnp.bfloat16, jnp.uint32
    S, D = x_v.shape
    F = w1_v.shape[1]
    dh = D // _H
    nt = D // _L
    nb = S // _BM
    hl = _L // 2

    def paced(keep, value, after):
        return jnp.where(keep, value, after)

    def keep_rows(n):
        return jnp.concatenate([one_s[...]] * (n // 8), axis=0) != 0

    def x_copy(i):
        rows = pl.ds(pl.multiple_of(i * _BM, _BM), _BM)
        return pltpu.make_async_copy(x_hbm.at[rows], x_v.at[rows], x_sem.at[i])

    wq_cp, wk_cp, wv_cp = [
        pltpu.make_async_copy(wqkv_hbm.at[:, pl.ds(j * D, D)], wqkv_v.at[j], w_sem.at[j])
        for j in range(3)]
    late_cp = [
        pltpu.make_async_copy(src, dst, w_sem.at[3 + j]) for j, (src, dst) in enumerate(
            ((w1_hbm, w1_v), (w2_hbm, w2_v), (wo_hbm, wo_v), (gw_hbm, gw_v)))]
    wk_cp.start()
    x_copy(0).start()
    qt_s[D // 2:D // 2 + hl, :] = jnp.zeros((hl, S), u32)
    s_s[1] = jnp.zeros((S, _BQ), f32)
    ev_s[...] = jnp.ones(ev_s.shape, f32)
    one_s[...] = jnp.ones(one_s.shape, jnp.int32)
    wk_cp.wait()

    def k_proj(i, carry):
        x_copy(i).wait()

        @pl.when(i < nb - 1)
        def _():
            x_copy(i + 1).start()

        pl.when(i == 0)(wq_cp.start)
        pl.when(i == 1)(wv_cp.start)
        pl.when(i == nb - 2)(wq_cp.wait)

        @pl.when(i == nb - 1)
        def _():
            wv_cp.wait()
            for cp in late_cp:
                cp.start()

        src = jnp.where(i == nb - 2, 0, jnp.where(i == nb - 1, 2, 1))
        wt_s[jnp.where(i == nb - 1, 1, 0)] = wqkv_v[src].T
        upper = lax.broadcasted_iota(jnp.int32, (_L, _L), 1) >= hl
        for a in range(_BM // _L):
            r0 = pl.multiple_of(i * _BM + a * _L, _L)
            pairs = pl.ds(pl.multiple_of(r0 // 2, hl), hl)
            k = _dot(x_v[pl.ds(r0, _L), :], wqkv_v[1])
            for j in range(nt):
                k_s[2 * j, pairs, :] = pltpu.bitcast(k[:, _tile(j)].astype(bf16), u32)
                if j + 1 < nt:
                    mixed = jnp.where(upper, k[:, _tile(j)], k[:, _tile(j + 1)])
                    k_s[2 * j + 1, pairs, :] = pltpu.bitcast(mixed.astype(bf16), u32)
        return carry

    lax.fori_loop(0, nb, k_proj, 0)

    def spread_keys(dst, rows, j, packed):
        for l in range(_L):
            col = jnp.broadcast_to(packed[:, l:l + 1], packed.shape)
            dst[j * _L + l, rows, :] = pltpu.bitcast(col, bf16).astype(f32)

    def qv_proj(i, carry):
        tok = pl.ds(pl.multiple_of(i * _BQV, _BQV), _BQV)
        xb = x_v[tok, :]
        n = 16 * pl.cdiv(_EARLY // 16, S // _BQV)
        e0 = pl.multiple_of(jnp.minimum(i * n, _EARLY - n), 16)
        for j in range(nt):
            spread_keys(ke_s, pl.ds(e0, n), j,
                        k_s[2 * j, pl.ds(pl.multiple_of(e0 // 2, 8), n // 2), :])
        v = _dot(wt_s[1], xb, _NT).astype(bf16).astype(f32)
        low = lax.broadcasted_iota(jnp.int32, (8, _BQV), 0) < 4
        for t in range(_H // 2):
            r = t * 2 * dh
            mid = v[r + 16:r + 24]
            vt_s[2 * t, :, tok] = jnp.concatenate(
                [v[r:r + 16], jnp.where(low, mid, 1.0)], axis=0)
            vt_s[2 * t + 1, :, tok] = jnp.concatenate(
                [jnp.where(low, 1.0, mid), v[r + 24:r + 40]], axis=0)
        scale = np.float32(dh ** -0.5 * np.log2(np.e))
        q = (_dot(wt_s[0], xb, _NT) * scale).astype(bf16)
        qt_s[0:D // 2, tok] = pltpu.bitcast(q, u32)
        qo_s[:, tok] = q.astype(f32)
        return carry

    lax.fori_loop(0, S // _BQV, qv_proj, 0)
    for cp in late_cp:
        cp.wait()

    fw = 4 * _L
    heads = _H // nb
    ek = _EARLY // 2
    e_steps = [(h, c, k0, d) for h in range(heads) for c in range(0, S // _L, 2)
               for k0 in range(0, _EARLY, ek) for d in range(dh)]
    n_dots = 2 * (F // fw) * nt
    e_cut = [len(e_steps) * min(j, n_dots - 1) // (n_dots - 1) for j in range(n_dots + 1)]

    def ffn(i, carry):
        rows = pl.ds(pl.multiple_of(i * _BM, _BM), _BM)
        state = {"dot": 0}

        def dot_and_scores(a, b):
            res = _dot(a, b)
            steps = e_steps[e_cut[state["dot"]]:e_cut[state["dot"] + 1]]
            state["dot"] += 1
            for n, (h, c, k0, d) in enumerate(steps):
                r = h * dh + d
                keys, cols = slice(k0, k0 + ek), slice(c * _L, (c + 2) * _L)
                if d == 0 or r % 8 == 0:
                    r8 = pl.multiple_of(i * heads * dh + r // 8 * 8, 8)
                    state["q"] = qo_s[pl.ds(r8, 8), cols]
                kd = ke_s[i * heads * dh + r, keys]
                if n % 4 == 0:
                    o = 8 * ((_BM - ek) // 8 * n // len(steps))
                    kd = paced(keep_rows(ek), kd, res[o:o + ek, 0:_L])
                term = jnp.concatenate([kd, kd], axis=1) * state["q"][r % 8:r % 8 + 1]
                state["s"] = term if d == 0 else state["s"] + term
                if d == dh - 1:
                    se_s[i * heads + h, keys, cols] = state["s"]
            return res

        hid = []
        for n in range(F // fw):
            rest = dot_and_scores(x_v[rows, fw:D], w1_v[fw:D, n * fw:(n + 1) * fw])
            cols = []
            for c in range(fw // _L):
                head = dot_and_scores(x_v[rows, 0:fw], w1_v[0:fw, _tile(n * fw // _L + c)])
                cols.append(jnp.maximum(head + rest[:, _tile(c)], 0.0).astype(bf16))
            hid.append(jnp.concatenate(cols, axis=1))
        nk = _VPU // nb
        v0 = pl.multiple_of(i * nk, nk)
        for j in range(nt):
            acc = None
            for n in range(F // fw):
                part = dot_and_scores(hid[n], w2_v[n * fw:(n + 1) * fw, _tile(j)])
                acc = part if n == 0 else acc + part
                if n == 0:
                    packed = k_s[2 * j, pl.ds(pl.multiple_of((_EARLY + v0) // 2, 8), nk // 2), :]
                    spread_keys(kb_s, pl.ds(v0, nk), j, paced(
                        keep_rows(nk // 2), packed, pltpu.bitcast(part[_BM - nk // 2:_BM], u32)))
            b_s[rows, _tile(j)] = acc
        return carry

    lax.fori_loop(0, nb, ffn, 0)

    nch = S // _KC
    nqt = _BQ // _L
    n_items = (S // _BQ) * _H
    first = _EARLY + _VPU
    k_cut = [first + 16 * ((S - first) // 16 * j // nch) for j in range(nch + 1)]
    v_steps = [(r, d) for r in range(0, _VPU, 8) for d in range(dh)]
    v_cut = [len(v_steps) * j // nch for j in range(nch + 1)]
    v_cut0 = [len(v_steps) * max(j - 2, 0) // (nch - 2) for j in range(nch + 1)]

    def queries(i):
        return pl.ds(pl.multiple_of((i // _H) * _BQ, _BQ), _BQ)

    def head_span(i):
        c0 = (i % _H) * dh
        j = c0 // _L
        lo = (c0 - j * _L) // 2
        return j, lo, lo + dh // 2

    def k_tile(i):
        j, _, hi = head_span(i)
        return 2 * j + (hi > hl).astype(jnp.int32)

    def mask_q(i, slot):
        j, lo, hi = head_span(i)
        r = pl.multiple_of(j * hl, hl)
        pair = lax.broadcasted_iota(jnp.int32, (hl, _BQ), 0)
        qm_s[slot] = jnp.where(
            (pair >= lo) & (pair < hi), qt_s[pl.ds(r, hl), queries(i)],
            jnp.where(pair < hi - hl, qt_s[pl.ds(r + hl, hl), queries(i)], u32(0)))

    def paced_rows(keep, value, after):
        return jnp.concatenate(
            [paced(keep, value[:, _tile(c)], after[8 * c:8 * c + 8, 0:_L]) for c in range(nqt)],
            axis=1)

    def spread_q(i, slot, dims, keep=None, after=None):
        base = ((i % _H) // 2) * 2 * dh
        for d in dims:
            r = slot * dh + d
            q8 = qo_s[pl.ds(pl.multiple_of(base + r // 8 * 8, 8), 8), queries(i)]
            if after is not None:
                q8 = paced_rows(keep, q8, after)
            qb_s[slot, d] = jnp.broadcast_to(q8[r % 8:r % 8 + 1], (8, _BQ))

    def put_scores(slot, r0, s, m):
        s_s[slot, r0:r0 + s.shape[0], :] = s
        top = jnp.max(s.reshape(s.shape[0] // 8, 8, _BQ), axis=0)
        return top if m is None else jnp.maximum(m, top)

    def probs_times_v(h, slot, j, m):
        keys = slice(j * _KC, (j + 1) * _KC)
        p = jnp.exp2(s_s[slot, keys, :] - m).astype(bf16)
        return _dot(vt_s[h, :, keys], p)

    def finish(i, odd_head, acc):
        if not odd_head:
            ev_s[...] = acc
            return
        even = ev_s[...] * (1.0 / ev_s[dh:dh + 1])
        odd = acc * (1.0 / acc[0:1])
        low = lax.broadcasted_iota(jnp.int32, (8, _BQ), 0) < 4
        r0 = pl.multiple_of(((i % _H) // 2) * 2 * dh, 8)
        qo_s[pl.ds(r0, 2 * dh), queries(i)] = jnp.concatenate(
            [even[0:16], jnp.where(low, even[16:24], odd[0:8]), odd[8:24]], axis=0)

    def attend(t, carry):
        m_in, kt = carry
        keep = keep_rows(8)
        maxes = [m_in]
        m = prev = part = acc = m_row = None
        for c in range(_ITEMS * nch + _LAG):
            if c < _ITEMS * nch:
                n, j = divmod(c, nch)
                i, slot = t * _ITEMS + n, n % 2
                nxt = jnp.minimum(i + 1, n_items - 1)
                if j == 0:
                    m = None
                cut = v_cut if n else v_cut0
                steps = v_steps[cut[j]:cut[j + 1]]
                for a, (r, d) in enumerate(steps):
                    kd = kb_s[(i % _H) * dh + d, r:r + 8, :]
                    if a % 3 == 0:
                        o = 8 * int(prev.shape[0] // 8 * (6 + 10 * a / len(steps)) / 16)
                        kd = paced(keep, kd, prev[o:o + 8, 0:_L])
                    term = jnp.concatenate([kd] * nqt, axis=1) * qb_s[slot, d]
                    part = term if d == 0 else part + term
                    if d == dh - 1:
                        m = put_scores(slot, _EARLY + r, part, m)
                if 4 <= j < 4 + dh // 2:
                    spread_q(nxt, 1 - slot, (2 * (j - 4), 2 * (j - 4) + 1), keep, prev)
                if 6 <= j < 6 + _EARLY // 8:
                    r = (j - 6) * 8
                    early = paced_rows(keep, se_s[i % _H, r:r + 8, queries(i)], prev)
                    m = put_scores(slot, r, early, m)
                if j == nch - 2:
                    mask_q(nxt, 1 - slot)
                k = pltpu.bitcast(k_s[kt, k_cut[j] // 2:k_cut[j + 1] // 2, :], bf16)
                prev = _dot(k, pltpu.bitcast(qm_s[slot], bf16))
                m = put_scores(slot, k_cut[j], prev, m)
                if j == nch - 1:
                    maxes.append(m)
                    kt = k_tile(nxt)
            if c >= _LAG:
                n, j = divmod(c - _LAG, nch)
                i = jnp.abs(t * _ITEMS + n - 1)
                if j == 0:
                    m_row = jnp.max(maxes[n], axis=0, keepdims=True)
                pv = probs_times_v(i % _H, 1 - n % 2, j, m_row)
                acc = pv if j == 0 else acc + pv
                if j == nch - 1:
                    finish(i, n % 2 == 0, acc)
        return maxes[_ITEMS], kt

    mask_q(jnp.int32(0), 0)
    spread_q(jnp.int32(0), 0, range(dh))
    m_last, _ = lax.fori_loop(
        0, n_items // _ITEMS, attend, (jnp.zeros((8, _BQ), f32), jnp.int32(0)))
    m_row = jnp.max(m_last, axis=0, keepdims=True)
    acc = att0 = None
    for j in range(nch):
        if j % 3 == 0 and j // 3 < nt:
            c = _tile(j // 3)
            part = _dot(qo_s[c, 0:_L].T.astype(bf16), wo_v[c, :])
            att0 = part if j == 0 else att0 + part
        pv = probs_times_v(_H - 1, 1, j, m_row)
        acc = pv if j == 0 else acc + pv
    finish(jnp.int32(n_items - 1), True, acc)

    out_cp = []
    for a in range(S // _L):
        rows = pl.ds(a * _L, _L)
        att = _dot(qo_s[:, rows].T.astype(bf16), wo_v[...]) if a else att0
        z = jnp.sum(x_v[rows, :].astype(f32) * gw_v[...].astype(f32), axis=-1, keepdims=True)
        gate = jax.nn.sigmoid(z)
        x_v[rows, :] = (gate * att + (1.0 - gate) * b_s[rows, :]).astype(x_v.dtype)
        out_cp.append(pltpu.make_async_copy(x_v.at[rows], o_hbm.at[rows], o_sem.at[a]))
        out_cp[-1].start()
    for cp in out_cp:
        cp.wait()


@jax.jit
def pallas_gated_mix__softmax_full_mha__dense_activation_relu__prompt_kernel(
    A_x: jax.Array,
    A_wqkv: jax.Array,
    A_wo: jax.Array,
    B_x: jax.Array,
    B_w1: jax.Array,
    B_w2: jax.Array,
    gate_w: jax.Array,
):
    del B_x
    B, S, D = A_x.shape
    F = B_w1.shape[1]
    assert (B, S, D, F) == (1, 2048, 640, 1536)
    bf16, f32, u32 = jnp.bfloat16, jnp.float32, jnp.uint32
    hbm = pl.BlockSpec(memory_space=pl.ANY)
    out = pl.pallas_call(
        _kernel,
        out_shape=jax.ShapeDtypeStruct((S, D), bf16),
        in_specs=[hbm] * 6,
        out_specs=hbm,
        scratch_shapes=[
            pltpu.VMEM((S, D), bf16),
            pltpu.VMEM((3, D, D), bf16),
            pltpu.VMEM((D, D), bf16),
            pltpu.VMEM((D, F), bf16),
            pltpu.VMEM((F, D), bf16),
            pltpu.VMEM((D,), bf16),
            pltpu.VMEM((2, D, D), bf16),
            pltpu.VMEM((2 * (D // _L) - 1, S // 2, _L), u32),
            pltpu.VMEM(((D + _L) // 2, S), u32),
            pltpu.VMEM((2, _L // 2, _BQ), u32),
            pltpu.VMEM((_H, _VROWS, S), f32),
            pltpu.VMEM((2, S, _BQ), f32),
            pltpu.VMEM((D, _VPU, _L), f32),
            pltpu.VMEM((D, _EARLY, _L), f32),
            pltpu.VMEM((_H, _EARLY, S), f32),
            pltpu.VMEM((D, S), f32),
            pltpu.VMEM((2, D // _H, 8, _BQ), f32),
            pltpu.VMEM((_VROWS, _BQ), f32),
            pltpu.VMEM((8, _L), jnp.int32),
            pltpu.VMEM((S, D), f32),
            pltpu.SemaphoreType.DMA((S // _BM,)),
            pltpu.SemaphoreType.DMA((7,)),
            pltpu.SemaphoreType.DMA((S // _L,)),
        ],
        compiler_params=pltpu.CompilerParams(vmem_limit_bytes=124 * 2**20),
    )(A_x.reshape(S, D), A_wqkv, A_wo, B_w1, B_w2, gate_w)
    return out.reshape(B, S, D)
```
